```python
import os as _os
_os.environ.setdefault('JAX_PLATFORMS', 'cpu')
import jax
import jax.numpy as jnp

def _softmax(x, axis=-1):
    return jax.nn.softmax(x, axis=axis)

def _gelu(x):
    return jax.nn.gelu(x, approximate=True)

def _silu(x):
    return jax.nn.silu(x)

def _sigmoid(x):
    return jax.nn.sigmoid(x)

def _layernorm(x, axis=-1, eps=1e-05):
    m = jnp.mean(x, axis=axis, keepdims=True)
    v = jnp.var(x, axis=axis, keepdims=True)
    return (x - m) / jnp.sqrt(v + eps)

def _scatter_add(tgt, idx, src, axis=0):
    return tgt.at[idx].add(src)

def _segment_sum(src, seg, n):
    return jax.ops.segment_sum(src, seg, n)

class _Rng:

    def __init__(self, key):
        self._k = key

    def _next(self):
        self._k, sub = jax.random.split(self._k)
        return sub

    def normal(self, shape):
        return jax.random.normal(self._next(), shape, dtype=jnp.bfloat16)

    def randint(self, lo, hi, shape):
        return jax.random.randint(self._next(), shape, lo, hi, dtype=jnp.int32)

    def uniform(self, shape, lo=0.0, hi=1.0):
        return jax.random.uniform(self._next(), shape, jnp.bfloat16, lo, hi)

    def permutation(self, n):
        return jax.random.permutation(self._next(), n)
kernel_name = 'adaLN_cond__memory_aug_recurrent_mem_tr__moe_arch_mod__prompt'

def setup_inputs():
    _rng = _Rng(jax.random.key(int.from_bytes(__import__("os").urandom(4), "little")))
    _w = lambda a: (lambda t: t.astype(jnp.bfloat16) if jnp.issubdtype(t.dtype, jnp.floating) else t)(jnp.asarray(a))

    def _A_setup():
        B, S, Dm = (1, 2048, 448)
        H, Dh = (16, 256)
        M, seg = (8, 32)
        seg = min(seg, S)
        S = S // seg * seg
        return {'x': _w((lambda *s: _rng.normal(s) * 0.05)(B, S, Dm)), 'mem0': _w((lambda *s: _rng.normal(s) * 0.4)(B, M, Dm)), 'Wq': _w((lambda *s: _rng.normal(s) * 1.6)(Dm, H, Dh) * Dm ** (-0.5)), 'Wk': _w((lambda *s: _rng.normal(s) * 1.6)(Dm, H, Dh) * Dm ** (-0.5)), 'Wv': _w((lambda *s: _rng.normal(s) * 0.4)(Dm, H, Dh) * Dm ** (-0.5)), 'Wo': _w((lambda *s: _rng.normal(s) * 0.4)(H, Dh, Dm) * (H * Dh) ** (-0.5)), 'seg_len': seg}
    _A_in = _A_setup()

    def _B_setup():
        B, S, D, F, C = (1, 2048, 448, 1792, 1)
        return {'x': _w((lambda *s: _rng.normal(s) * 0.05)(B, S, D)), 'w_r': _w((lambda *s: _rng.normal(s) * 0.05)(D)), 'w_gate': _w((lambda *s: _rng.normal(s) * 0.05)(D, F)), 'w_up': _w((lambda *s: _rng.normal(s) * 0.05)(D, F)), 'w_down': _w((lambda *s: _rng.normal(s) * 0.05)(F, D))}
    _B_in = _B_setup()
    return {'A_x': _A_in['x'], 'A_mem0': _A_in['mem0'], 'A_Wq': _A_in['Wq'], 'A_Wk': _A_in['Wk'], 'A_Wv': _A_in['Wv'], 'A_Wo': _A_in['Wo'], 'A_seg_len': _A_in['seg_len'], 'B_x': _B_in['x'], 'B_w_r': _B_in['w_r'], 'B_w_gate': _B_in['w_gate'], 'B_w_up': _B_in['w_up'], 'B_w_down': _B_in['w_down'], 'c': _w((lambda *s: _rng.normal(s) * 0.05)(1, 448) * 8.0), 'w_mod': _w((lambda *s: _rng.normal(s) * 0.05)(448, 6 * 448) * 448 ** (-0.5) * 8.0)}

def reference(A_x, A_mem0, A_Wq, A_Wk, A_Wv, A_Wo, A_seg_len, B_x, B_w_r, B_w_gate, B_w_up, B_w_down, c, w_mod):

    def _A_ref(x, mem0, Wq, Wk, Wv, Wo, seg_len):
        B, S, Dm = x.shape
        H, Dh = (Wq.shape[1], Wq.shape[2])
        M = mem0.shape[1]
        scale = Dh ** (-0.5)
        n_seg = S // seg_len
        L = M + seg_len
        idx = jnp.arange(L)
        mask = (idx[:, None] < M) | (idx[:, None] >= idx[None, :])
        mem = mem0
        outs = []
        for s in range(n_seg):
            xs = x[:, s * seg_len:(s + 1) * seg_len, :].copy()
            h = jnp.concatenate([mem, xs], axis=1)
            q = jnp.einsum('btd,dhe->bhte', h, Wq)
            k = jnp.einsum('btd,dhe->bhte', h, Wk)
            v = jnp.einsum('btd,dhe->bhte', h, Wv)
            scores = jnp.einsum('bhqe,bhke->bhqk', q, k) * scale
            scores = jnp.where(mask[None, None], scores, -1000000000.0)
            p = _softmax(scores, axis=-1)
            o = jnp.einsum('bhqk,bhke->bhqe', p, v)
            o = jnp.einsum('bhte,hed->btd', o, Wo)
            mem = o[:, :M, :].copy()
            outs.append(o[:, M:, :])
        return jnp.concatenate(outs, axis=1)

    def _B_ref(x, w_r, w_gate, w_up, w_down):
        B, S, D = x.shape
        C = 1
        r = x @ w_r
        idx = jnp.argsort(-r, axis=-1)[:, :C]
        idx_e = jnp.repeat(idx.reshape(B, C, 1), D, axis=2)
        x_sel = jnp.take_along_axis(x, idx_e, axis=1)
        g = _silu(x_sel @ w_gate)
        u = x_sel @ w_up
        y = g * u @ w_down
        r_sel = _sigmoid(jnp.take_along_axis(r, idx, axis=1))
        y = y * r_sel.reshape(B, C, 1)
        b_off = (jnp.arange(B) * S).reshape(B, 1)
        flat_idx = (idx + b_off).reshape(B * C)
        zero = (x * 0.0).reshape(B * S, D)
        upd = _scatter_add(zero, flat_idx, y.reshape(B * C, D), axis=0)
        return x + upd.reshape(B, S, D)
    x = A_x
    mod = (_silu(c) @ w_mod).reshape(c.shape[0], 6, 1, -1)
    sa, ca, ga, sb, cb, gb = (mod[:, 0].copy(), mod[:, 1].copy(), mod[:, 2].copy(), mod[:, 3].copy(), mod[:, 4].copy(), mod[:, 5].copy())
    h = _layernorm(x, axis=-1) * (1 + ca) + sa
    x = x + ga * _A_ref(h, A_mem0, A_Wq, A_Wk, A_Wv, A_Wo, A_seg_len)
    h = _layernorm(x, axis=-1) * (1 + cb) + sb
    x = x + gb * _B_ref(h, B_w_r, B_w_gate, B_w_up, B_w_down)
    return x
```

```python
import functools

import jax
import jax.numpy as jnp
import jax.experimental.pallas as pl
import jax.experimental.pallas.tpu as pltpu

F32 = jnp.float32
BF16 = jnp.bfloat16
LANES = 128
D_MODEL = 448
N_SEMS = 32
NT = (((1,), (1,)), ((), ()))
AHEAD = 2
AHEAD0 = 0
SIDE0 = 8
LEAD3 = 1
V_SPLIT = 12


def _rb(t):
    return t.astype(BF16).astype(F32)


def _words(t):
    return pltpu.bitcast(t.astype(BF16), jnp.uint32)


def _halves(t):
    return pltpu.bitcast(t, BF16)


def _ln_stats(load):
    n = D_MODEL
    mean = jnp.sum(load(), axis=0, keepdims=True) / n
    cen = load() - mean
    var = jnp.sum(cen * cen, axis=0, keepdims=True) / n
    return _rb(mean), 1.0 / _rb(jnp.sqrt(_rb(_rb(var) + 1e-5)))


def _group8_allreduce(v, op, lane):
    for d in (1, 2, 4):
        v = op(v, jnp.where((lane & d) != 0, pltpu.roll(v, d, 1), pltpu.roll(v, LANES - d, 1)))
    return v


def _kernel(c_hbm, mem0_hbm, wr_hbm,
            xt_hbm, wq_hbm, wk_hbm, wv_hbm, wot_hbm, wg_hbm, wu_hbm, wdt_hbm, wmod_hbm,
            out_hbm,
            c_ref, mem0_ref, wr_ref, xt_v, raw_v, a_v, k_v, q0_v, q1_v, q2_v, q3_v, wot_v, w_v, wg_v, wu_v, wdt_v, wmod_v,
            modb_v, h_v, o_v, x1_v, z0_v, z1_v, v_v, r_v, out_v, sems,
            *, seg, scale):
    q_v = (q0_v, q1_v, q2_v, q3_v)
    z_v = (z0_v, z1_v)
    d_model, seq = xt_v.shape
    n_mem = mem0_ref.shape[0]
    n_heads = wot_v.shape[0]
    n_pair = n_heads // 2
    n_blk = seq // LANES
    per_blk = LANES // seg
    n_main = d_model // LANES
    d_main = n_main * LANES
    half = d_model - d_main
    rows = n_mem + seg
    n_grp = rows // 8

    tiles = [(lo, min(lo + LANES, d_model)) for lo in range(0, d_model, LANES)]
    n_tile = len(tiles)

    sem_ids = iter(range(N_SEMS))

    def copy(src, dst):
        return pltpu.make_async_copy(src, dst, sems.at[next(sem_ids)])

    def row_chunks(src, dst):
        return [copy(src.at[lo:hi], dst.at[lo:hi]) for lo, hi in tiles]

    cp_wk = row_chunks(wk_hbm, raw_v.at[1])
    cp_wq = row_chunks(wq_hbm, raw_v.at[2])
    cp_wv = copy(wv_hbm, raw_v.at[0])
    wot_cuts = (0, 1, 4, 6, n_pair)
    cp_wot = [copy(wot_hbm.at[2 * lo:2 * hi], wot_v.at[2 * lo:2 * hi]) for lo, hi in zip(wot_cuts, wot_cuts[1:])]
    cp_mod = [copy(wmod_hbm, wmod_v), copy(c_hbm, c_ref), copy(mem0_hbm, mem0_ref), copy(wr_hbm, wr_ref)]
    cp_x = [copy(xt_hbm.at[:, lo:hi], xt_v.at[:, lo:hi]) for lo, hi in ((0, 2 * LANES), (2 * LANES, seq))]
    cp_ffn = [copy(wg_hbm, wg_v), copy(wu_hbm, wu_v), copy(wdt_hbm, wdt_v)]
    for cp in cp_wk + cp_wq + cp_wot[:1] + [cp_wv] + cp_wot[1:] + cp_mod + cp_x + cp_ffn:
        cp.start()
    out_sem = next(sem_ids)

    def out_copy(b):
        return pltpu.make_async_copy(out_v.at[0, b], out_hbm.at[:, pl.ds(pl.multiple_of(b * LANES, LANES), LANES)],
                                     sems.at[out_sem])

    def split_rows(which, dst, r0, d0):
        dst[:, d0:d0 + 16, :] = jnp.swapaxes(raw_v[which, r0:r0 + 16], 0, 1)

    def split_jobs(which, dst, t, base=0):
        lo, hi = tiles[t]
        return [functools.partial(split_rows, which, dst, r0, r0 - base) for r0 in range(lo, hi, 16)]

    low = jax.lax.broadcasted_iota(jnp.int32, (d_model, LANES), 1) < half

    def fold(which, a_ref, b_rows, p, t, mult):
        if t < n_main:
            for k in range(2):
                res = jax.lax.dot_general(a_ref[2 * p + k], b_rows(2 * p + k), NT, preferred_element_type=F32)
                w_v[which, p, 2 * t + k] = _words(res * mult)
        else:
            tails = jnp.concatenate([b_rows(2 * p), b_rows(2 * p + 1)], axis=0)
            res = [jax.lax.dot_general(a_ref[2 * p + k], tails, NT, preferred_element_type=F32) for k in range(2)]
            w_v[which, p, 2 * n_main] = _words(jnp.where(low, res[0], res[1]) * mult)

    def value_jobs(p):
        return [functools.partial(fold, 1, a_v, lambda h, lo=lo, hi=hi: wot_v[h, lo:hi, :], p, t, 1.0)
                for t, (lo, hi) in enumerate(tiles)]

    def key_jobs(t):
        lo, hi = tiles[t]
        return [functools.partial(fold, 0, k_v, lambda h: q_v[t][h, 0:hi - lo, :], p, t, scale)
                for p in range(n_pair)]

    def run(*job_lists):
        for jobs in job_lists:
            for job in jobs:
                job()

    lead = 3
    for t in range(n_tile):
        cp_wk[t].wait()
        run(split_jobs(1, k_v, t))
    cp_wq[0].wait()
    run(split_jobs(2, q_v[0], 0), key_jobs(0)[:lead])
    cp_wq[1].wait()
    run(key_jobs(0)[lead:], split_jobs(2, q_v[1], 1, tiles[1][0]), key_jobs(1)[:lead])
    cp_wq[2].wait()
    cp_wq[3].wait()
    run(key_jobs(1)[lead:], split_jobs(2, q_v[2], 2, tiles[2][0]), key_jobs(2),
        split_jobs(2, q_v[3], 3, tiles[3][0]), key_jobs(3)[:LEAD3])
    cp_wot[0].wait()
    cp_wv.wait()
    run(key_jobs(3)[LEAD3:], *[split_jobs(0, a_v, t) for t in range(n_tile)], value_jobs(0))
    for i in (1, 2, 3):
        cp_wot[i].wait()
        if i == 3:
            for cp in cp_mod + cp_x[:1]:
                cp.wait()
        run(*[value_jobs(p) for p in range(wot_cuts[i], wot_cuts[i + 1])])

    cv = c_ref[...].astype(F32)
    sc = _rb(cv * _rb(jax.nn.sigmoid(cv)))
    mod = _rb(jnp.dot(jnp.broadcast_to(sc, (8, d_model)), wmod_v[...], preferred_element_type=F32))
    for t in range(mod.shape[1] // LANES):
        tile = jnp.broadcast_to(mod[0:1, t * LANES:(t + 1) * LANES], (LANES, LANES))
        modb_v[t * LANES:(t + 1) * LANES, :] = tile.T
    for k in (1, 4):
        modb_v[k * d_model:(k + 1) * d_model, :] = _rb(1.0 + modb_v[k * d_model:(k + 1) * d_model, :])

    def row_to_col(row):
        wide = jnp.concatenate([row, jnp.zeros((1, half), F32)], axis=1)
        return jnp.broadcast_to(wide, (LANES, d_model + half)).T[:d_model]

    modb_v[6 * d_model:7 * d_model, :] = row_to_col(wr_ref[...].astype(F32).reshape(1, d_model))

    def modv(k, lo=0, hi=d_model):
        return modb_v[k * d_model + lo:k * d_model + hi, :]

    def x_rows(b, lo=0, hi=d_model):
        return xt_v[lo:hi, pl.ds(pl.multiple_of(b * LANES, LANES), LANES)].astype(F32)

    def pre_jobs(b, row0):
        stats = []

        def moments():
            stats.extend(_ln_stats(lambda: x_rows(b)))
            return jnp.broadcast_to(stats[1], (8, LANES))

        def tile(lo, hi):
            h = (x_rows(b, lo, hi) - stats[0]) * stats[1] * modv(1, lo, hi) + modv(0, lo, hi)
            if hi - lo < LANES:
                h = jnp.concatenate([h, h], axis=0)
            h_v[row0:row0 + LANES, lo:lo + LANES] = h.T
            return h_v[row0 + LANES - 8:row0 + LANES, lo:lo + LANES]

        return [moments] + [functools.partial(tile, lo, hi) for lo, hi in tiles]

    def emit(x1, h2, upd, lo=0, hi=d_model):
        return (x1 + modv(5, lo, hi) * (h2 + upd)).astype(BF16)

    def post_jobs(b, b_again):
        stats = []
        score = [jnp.zeros((8, LANES), F32)]

        def residual(lo, hi):
            x1_v[b, lo:hi, :] = x_rows(b, lo, hi) + modv(2, lo, hi) * o_v[:, lo:lo + LANES].T[:hi - lo]
            return x1_v[b_again, hi - 8:hi, :]

        def moments():
            stats.extend(_ln_stats(lambda: x1_v[b_again]))
            return jnp.broadcast_to(stats[1], (8, LANES))

        def chunk(lo, hi):
            x1 = x1_v[b_again, lo:hi, :]
            h2 = (x1 - stats[0]) * stats[1] * modv(4, lo, hi) + modv(3, lo, hi)
            part = h2 * modv(6, lo, hi)
            score[0] = score[0] + (part[0:8] + part[8:16]) + (part[16:24] + part[24:32])
            out_v[0, b, lo:hi, :] = emit(x1, h2, h2 * 0.0, lo, hi)
            out_v[1, b, lo:hi, :] = h2.astype(BF16)
            if hi == d_model:
                r_v[pl.ds(b, 1), :] = jnp.sum(score[0], axis=0, keepdims=True)
            return pltpu.bitcast(out_v[0, b_again, lo:lo + 16, :], F32)

        return ([functools.partial(residual, lo, hi) for lo, hi in tiles] + [moments]
                + [functools.partial(chunk, lo, lo + 32) for lo in range(0, d_model, 32)])

    lane8 = jax.lax.broadcasted_iota(jnp.int32, (8, LANES), 1)
    low8 = lane8 < half
    causal = jax.lax.broadcasted_iota(jnp.int32, (8, LANES), 0) >= lane8 % 8

    def project(lhs, which, p, t, dsts, after=None):
        if after is not None:
            always = (pltpu.bitcast(after, jnp.int32) | 1) != 0
            first = jnp.concatenate([jnp.where(always, lhs[:8, :LANES], 0.0), lhs[:8, LANES:]], axis=1)
            lhs = jnp.concatenate([first, lhs[8:]], axis=0)
        if t < n_main:
            w = jnp.concatenate([_halves(w_v[which, p, 2 * t]), _halves(w_v[which, p, 2 * t + 1])], axis=1)
        else:
            w = _halves(w_v[which, p, 2 * n_main])
        y = jnp.dot(lhs[:, :d_model], w, preferred_element_type=F32)
        for i, (dst, g) in enumerate(dsts):
            yg = y[8 * i:8 * i + 8]
            if t < n_main:
                pair = [yg[:, :LANES], yg[:, LANES:]]
            else:
                pair = [jnp.where(low8, yg, 0.0), jnp.where(low8, 0.0, yg)]
            r0 = g * 4 * n_heads + 8 * p
            dst[t, r0:r0 + 8, :] = _words(jnp.concatenate(pair, axis=0))

    def tokens(start, count):
        dsts = [(z_v[(r // seg) % 2], 1 + (r % seg) // 8) for r in range(start, start + count, 8)]
        return h_v[start:start + count, :], dsts

    key_tiles = [(p, t) for t in range(n_tile) for p in range(n_pair)]
    ahead = {tile: i % per_blk for i, tile in enumerate(key_tiles[AHEAD0:AHEAD0 + AHEAD * per_blk])}

    def run_ahead(q, group):
        lhs, dsts = tokens(q * seg, seg)
        for (p, t), k in ahead.items():
            if k == group:
                project(lhs, 0, p, t, dsts)

    def step(q, mem, side):
        z_cur = z_v[q % 2]
        tok, dsts = tokens(q * seg, seg)
        t_ext = jnp.concatenate([mem, tok], axis=0)
        side = list(side)
        for i, (p, t) in enumerate(key_tiles):
            if (p, t) in ahead:
                phase = (q - ahead[p, t]) % per_blk
                part, part_dsts = tokens((q + 1) * seg - 8 * phase, seg - 8)
                project(jnp.concatenate([mem, part], axis=0), 0, p, t, [(z_cur, 0)] + part_dsts)
            else:
                after = side.pop(0)() if side and i >= SIDE0 else None
                project(t_ext, 0, p, t, [(z_cur, 0)] + dsts, after)
        assert not side
        v_order = [(p, t) for t in (n_main, *range(n_main)) for p in range(n_pair)]
        v_dsts = [(v_v, g) for g in range(n_grp)]
        for p, t in v_order[:V_SPLIT]:
            project(t_ext, 1, p, t, v_dsts)
        keys_t = jnp.concatenate(
            [jnp.concatenate([_halves(z_cur[t, g * (LANES // 2):(g + 1) * (LANES // 2), :]).T
                              for g in range(n_grp)], axis=1) for t in range(n_tile)], axis=0)
        sco = jnp.dot(t_ext, keys_t, preferred_element_type=F32)
        probs = []
        for rg in range(n_grp):
            parts = []
            for g in range(n_grp):
                part = sco[8 * rg:8 * rg + 8, g * LANES:(g + 1) * LANES]
                if 0 < rg == g:
                    part = jnp.where(causal, part, -1e9)
                elif 0 < rg < g:
                    part = jnp.full_like(part, -1e9)
                parts.append(part)
            top = _group8_allreduce(functools.reduce(jnp.maximum, parts), jnp.maximum, lane8)
            ex = [jnp.exp(part - top) for part in parts]
            inv = 1.0 / _group8_allreduce(functools.reduce(jnp.add, ex), jnp.add, lane8)
            probs.append(jnp.concatenate([e * inv for e in ex], axis=1))
        for p, t in v_order[V_SPLIT:]:
            project(t_ext, 1, p, t, v_dsts)
        prob = jnp.concatenate(probs, axis=0)
        tail = jnp.dot(prob, _halves(v_v[n_main]), preferred_element_type=F32)
        outs = [jnp.dot(prob, _halves(v_v[t]), preferred_element_type=F32) for t in range(n_main)]
        o = jnp.concatenate(outs + [tail + pltpu.roll(tail, half, 1)], axis=1)
        o_v[q * seg:(q + 1) * seg, :] = o[n_mem:]
        run_ahead(q + 1, (q + 1) % per_blk)
        return o[:n_mem]

    def block(b, mem):
        post = post_jobs(jnp.maximum(b - 1, 0), b - jnp.minimum(b, 1))
        nxt = pre_jobs(jnp.minimum(b + 1, n_blk - 1), LANES)
        side = [nxt[:1] + post[:5], post[5:], [], []]
        for q in range(per_blk):
            mem = step(q, mem, side[q])
            if q == 0:
                run(nxt[1:])
        h_v[:LANES] = h_v[LANES:]

        @pl.when(b == 0)
        def _():
            cp_x[1].wait()

        @pl.when(b > 0)
        def _():
            out_copy(b - 1).start()
        return mem

    run(pre_jobs(0, 0))
    for k in range(per_blk):
        run_ahead(0, k)
    o_v[...] = jnp.zeros(o_v.shape, F32)
    m0 = mem0_ref[...].astype(F32)
    jax.lax.fori_loop(0, n_blk, block, jnp.concatenate([m0, m0[:, d_main:]], axis=1))
    run(post_jobs(n_blk - 1, n_blk - 1))
    out_copy(n_blk - 1).start()

    r = _rb(r_v[...])
    r = jnp.where(r != r, -jnp.inf, r)
    best = jnp.max(r, keepdims=True)
    pos = (jax.lax.broadcasted_iota(jnp.int32, r.shape, 0) * LANES
           + jax.lax.broadcasted_iota(jnp.int32, r.shape, 1))
    idx = jnp.min(jnp.where(r == best, pos, seq - 1))
    blk = idx // LANES
    x1 = x1_v[blk]
    h2 = out_v[1, blk].astype(F32)
    hit = jax.lax.broadcasted_iota(jnp.int32, h2.shape, 1) == idx % LANES
    col = jnp.sum(jnp.where(hit, h2, 0.0), axis=1, keepdims=True)
    col = jnp.concatenate([jnp.broadcast_to(col, (d_model, LANES)), jnp.zeros((half, LANES), F32)], axis=0)
    sel = col.T[:8, :d_model]
    for cp in cp_ffn:
        cp.wait()
    gate = _rb(jnp.dot(sel, wg_v[...], preferred_element_type=F32))
    up = _rb(jnp.dot(sel, wu_v[...], preferred_element_type=F32))
    act = _rb(_rb(gate * _rb(jax.nn.sigmoid(gate))) * up)
    y = _rb(jax.lax.dot_general(act, wdt_v[...], NT, preferred_element_type=F32))
    y = _rb(y[0:1] * _rb(jax.nn.sigmoid(best)))
    zero = h2 * 0.0
    for b in range(n_blk):
        out_copy(b).wait()
    out_v[0, blk] = emit(x1, h2, jnp.where(hit, _rb(zero + row_to_col(y)), zero))
    out_copy(blk).start()
    out_copy(blk).wait()


@functools.partial(jax.jit, static_argnames=("A_seg_len",))
def pallas_adaLN_cond__memory_aug_recurrent_mem_tr__moe_arch_mod__prompt_kernel(
    A_x, A_mem0, A_Wq, A_Wk, A_Wv, A_Wo, A_seg_len, B_x, B_w_r, B_w_gate, B_w_up, B_w_down, c, w_mod,
):
    del B_x
    _, seq, d_model = A_x.shape
    n_mem = A_mem0.shape[1]
    n_heads, d_head = A_Wq.shape[1:]
    d_ff = B_w_gate.shape[1]
    seg = int(A_seg_len)
    rows = n_mem + seg
    d_ext = d_model + LANES // 2
    assert A_x.shape[0] == 1 and d_model % LANES == LANES // 2 and n_mem == 8
    assert n_heads * 8 == LANES and seg % 8 == 0 and seq % LANES == 0 and LANES % seg == 0

    hbm = pl.BlockSpec(memory_space=pltpu.HBM)
    out_t = pl.pallas_call(
        functools.partial(_kernel, seg=seg, scale=d_head ** -0.5),
        out_shape=jax.ShapeDtypeStruct((d_model, seq), A_x.dtype),
        in_specs=[hbm] * 12,
        out_specs=hbm,
        scratch_shapes=[
            pltpu.VMEM(c.shape, BF16),
            pltpu.VMEM((n_mem, d_model), BF16),
            pltpu.VMEM(B_w_r.shape, BF16),
            pltpu.VMEM((d_model, seq), BF16),
            pltpu.VMEM((3, d_model, n_heads, d_head), BF16),
            pltpu.VMEM((n_heads, d_model, d_head), BF16),
            pltpu.VMEM((n_heads, d_model, d_head), BF16),
            *[pltpu.VMEM((n_heads, LANES, d_head), BF16)] * 4,
            pltpu.VMEM((n_heads, d_model, d_head), BF16),
            pltpu.VMEM((2, n_heads // 2, 2 * d_model // LANES, d_model // 2, LANES), jnp.uint32),
            pltpu.VMEM((d_model, d_ff), BF16),
            pltpu.VMEM((d_model, d_ff), BF16),
            pltpu.VMEM((d_model, d_ff), BF16),
            pltpu.VMEM(w_mod.shape, BF16),
            pltpu.VMEM((7 * d_model, LANES), F32),
            pltpu.VMEM((2 * LANES, d_ext), F32),
            pltpu.VMEM((LANES, d_ext), F32),
            pltpu.VMEM((seq // LANES, d_model, LANES), F32),
            *[pltpu.VMEM((d_ext // LANES, rows * n_heads // 2, LANES), jnp.uint32)] * 2,
            pltpu.VMEM((d_ext // LANES, rows * n_heads // 2, LANES), jnp.uint32),
            pltpu.VMEM((seq // LANES, LANES), F32),
            pltpu.VMEM((2, seq // LANES, d_model, LANES), BF16),
            pltpu.SemaphoreType.DMA((N_SEMS,)),
        ],
        compiler_params=pltpu.CompilerParams(vmem_limit_bytes=100 * 1024 * 1024),
    )(c, A_mem0[0], B_w_r,
      A_x[0].T, A_Wq, A_Wk, A_Wv, jnp.swapaxes(A_Wo, 1, 2), B_w_gate, B_w_up, B_w_down.T, w_mod)
    return out_t.T[None]
```

```python
import functools

import jax
import jax.numpy as jnp
import jax.experimental.pallas as pl
import jax.experimental.pallas.tpu as pltpu

F32 = jnp.float32
BF16 = jnp.bfloat16
LANES = 128
NT = (((1,), (1,)), ((), ()))

AHEAD = 3
AHEAD_FIRST = 8
VALUES_EARLY = 12
MOD_PAD = 16


def _rb(t):
    return t.astype(BF16).astype(F32)


def _load16(ref, lo=None, hi=None):
    words = ref.bitcast(jnp.uint32)
    return pltpu.bitcast(words[...] if lo is None else words[lo // 2:hi // 2], BF16)


def _after(t, token):
    always = (pltpu.bitcast(jnp.broadcast_to(token, (8, LANES)), jnp.int32) | 1) != 0
    top = jnp.concatenate([jnp.where(always, t[:8, :LANES], 0.0), t[:8, LANES:]], axis=1)
    return jnp.concatenate([top, t[8:]], axis=0)


def _ln_stats(load):
    x = load()
    n = x.shape[0]
    mean = jnp.sum(x, axis=0, keepdims=True) / n
    cen = load() - mean
    var = jnp.sum(cen * cen, axis=0, keepdims=True) / n
    return _rb(mean), 1.0 / _rb(jnp.sqrt(_rb(_rb(var) + 1e-5)))


def _group8_allreduce(v, op, lane):
    for d in (1, 2, 4):
        v = op(v, jnp.where((lane & d) != 0, pltpu.roll(v, d, 1), pltpu.roll(v, LANES - d, 1)))
    return v


def _kernel(c_hbm, mem0_hbm, wr_hbm, xt_hbm, wq_hbm, wk_hbm, wv_hbm, wot_hbm, wg_hbm, wu_hbm, wdt_hbm, wmod_hbm,
            out_hbm,
            c_v, mem0_v, wr_v, xt_v, pair_v, wot_v, w_v, wg_v, wu_v, wdt_v, wmod_v,
            mod_v, h_v, o_v, x1_v, key0_v, key1_v, val_v, r_v, y_v, h2_v, out_v, sems,
            *, seg, scale):
    key_v = (key0_v, key1_v)
    d_model, seq = xt_v.shape
    n_mem = mem0_v.shape[0]
    n_heads, n_head_tile = wot_v.shape[:2]
    n_pair = n_heads // 2
    n_blk = seq // LANES
    per_blk = LANES // seg
    n_main = d_model // LANES
    d_main = n_main * LANES
    half = d_model - d_main
    n_grp = (n_mem + seg) // 8
    tiles = [(lo, min(lo + LANES, d_model)) for lo in range(0, d_model, LANES)]
    n_tile = len(tiles)

    sem_ids = iter(range(sems.shape[0]))

    def copies(*pairs):
        sem = sems.at[next(sem_ids)]
        return [pltpu.make_async_copy(src, dst, sem) for src, dst in pairs]

    def wait(group):
        for cp in group:
            cp.wait()

    def head_pair(src, which, p):
        return src.bitcast(jnp.uint32).at[:, p, :], pair_v.at[which, p]

    first = slice(0, 2 * d_model)
    later = slice(2 * d_model, 6 * d_model)
    cp_val = [copies(head_pair(wv_hbm, 0, p),
                     *[(wot_hbm.at[2 * p:2 * p + 2, :, e * LANES:(e + 1) * LANES], wot_v.at[2 * p:2 * p + 2, e])
                       for e in range(n_head_tile)]) for p in range(n_pair)]
    cp_key = [copies(head_pair(wk_hbm, 1, p), head_pair(wq_hbm, 2, p)) for p in range(n_pair)]
    cp_first = copies((c_hbm, c_v), (mem0_hbm, mem0_v), (wr_hbm, wr_v), (wmod_hbm.at[:, first], wmod_v.at[:, first]),
                      (xt_hbm.at[:, :LANES], xt_v.at[:, :LANES]))
    cp_second = copies((xt_hbm.at[:, LANES:2 * LANES], xt_v.at[:, LANES:2 * LANES]))
    cp_later = copies((wmod_hbm.at[:, later], wmod_v.at[:, later]), (xt_hbm.at[:, 2 * LANES:], xt_v.at[:, 2 * LANES:]))
    cp_ffn = copies((wg_hbm, wg_v), (wu_hbm, wu_v), (wdt_hbm, wdt_v))
    for cp in sum(cp_val + cp_key, []) + cp_first + cp_second + cp_later + cp_ffn:
        cp.start()
    out_sem = next(sem_ids)

    def out_copy(b):
        return pltpu.make_async_copy(out_v.at[b], out_hbm.at[:, pl.ds(pl.multiple_of(b * LANES, LANES), LANES)],
                                     sems.at[out_sem])

    mod_v[2:6] = jnp.zeros((4, *mod_v.shape[1:]), F32)
    o_v[...] = jnp.zeros(o_v.shape, F32)

    def pair_rows(which, p, k, lo, hi):
        words = pair_v[which, p, lo:hi, :]
        return pltpu.bitcast(words << 16 if k == 0 else words & jnp.uint32(0xFFFF0000), F32)

    def wo_rows(p, k, lo, hi):
        return jnp.concatenate([_load16(wot_v.at[2 * p + k, e], lo, hi) for e in range(n_head_tile)], axis=1)

    def fold(which, p, a_rows, b_rows, mult):
        def product(u, v):
            return jax.lax.dot_general(u, v.astype(BF16), NT, preferred_element_type=F32)

        tail = jnp.concatenate([product(b_rows(p, k, d_main, d_model), a_rows(p, k, 0, d_model))
                                for k in range(2)], axis=0)
        tail = jnp.concatenate([tail, jnp.zeros((LANES, half), F32)], axis=1).T[:d_model]
        w_v[which, p, 2 * n_main] = (tail * mult).astype(BF16)
        for t in range(n_main):
            for k in range(2):
                res = product(a_rows(p, k, 0, d_model), b_rows(p, k, t * LANES, (t + 1) * LANES))
                w_v[which, p, 2 * t + k] = (res * mult).astype(BF16)

    for p in range(n_pair):
        wait(cp_val[p])
        fold(1, p, functools.partial(pair_rows, 0), wo_rows, 1.0)
    for p in range(n_pair):
        wait(cp_key[p])
        fold(0, p, functools.partial(pair_rows, 1), functools.partial(pair_rows, 2), scale)

    def modulation(cols):
        cv = c_v[...].astype(F32)
        act = _rb(cv * _rb(jax.nn.sigmoid(cv)))
        mod = _rb(jnp.dot(jnp.broadcast_to(act, (8, d_model)), wmod_v[:, cols], preferred_element_type=F32))
        for c0 in range(0, mod.shape[1], LANES):
            tile = jnp.broadcast_to(mod[0:1, c0:c0 + LANES], (LANES, LANES)).T
            for r in range(0, LANES, half):
                k, lo = divmod(cols.start + c0 + r, d_model)
                part = tile[r:r + half]
                mod_v[k, lo:lo + half, :] = _rb(1.0 + part) if k in (1, 4) else part

    wait(cp_first)
    modulation(first)
    router = jnp.concatenate([wr_v[...].astype(F32).reshape(1, d_model), jnp.zeros((1, half), F32)], axis=1)
    mod_v[6, :d_model, :] = jnp.broadcast_to(router, (LANES, d_model + half)).T[:d_model]
    shift_a, scale_a, gate_a, shift_b, scale_b, gate_b, w_router = range(7)

    def x_rows(b, lo=0, hi=d_model):
        return xt_v[lo:hi, pl.ds(pl.multiple_of(b * LANES, LANES), LANES)].astype(F32)

    def pre(b, row0):
        stats = []

        def moments():
            stats.extend(_ln_stats(lambda: x_rows(b)))
            return stats[1]

        def rest():
            for lo, hi in tiles:
                h = (x_rows(b, lo, hi) - stats[0]) * stats[1] * mod_v[scale_a, lo:hi] + mod_v[shift_a, lo:hi]
                if hi - lo < LANES:
                    h = jnp.concatenate([h, h], axis=0)
                h_v[row0:row0 + LANES, lo:lo + LANES] = h.T

        return moments, rest

    def emit(x1, h2, upd, lo=0, hi=d_model):
        return (x1 + mod_v[gate_b, lo:hi] * (h2 + upd)).astype(BF16)

    def post(b, b_again):
        stats = []

        def residual():
            for lo, hi in tiles:
                x1_v[b, lo:hi, :] = x_rows(b, lo, hi) + mod_v[gate_a, lo:hi] * o_v[:, lo:lo + LANES].T[:hi - lo]

        def moments():
            stats.extend(_ln_stats(lambda: x1_v[b_again]))
            return stats[1]

        def rest():
            score = jnp.zeros((8, LANES), F32)
            for lo in range(0, d_model, 32):
                hi = lo + 32
                x1 = x1_v[b_again, lo:hi, :]
                h2 = (x1 - stats[0]) * stats[1] * mod_v[scale_b, lo:hi] + mod_v[shift_b, lo:hi]
                part = h2 * mod_v[w_router, lo:hi]
                score = score + (part[0:8] + part[8:16]) + (part[16:24] + part[24:32])
                out_v[b, lo:hi, :] = emit(x1, h2, h2 * 0.0, lo, hi)
                h2_v[b, lo:hi, :] = h2.astype(BF16)
            r_v[pl.ds(b, 1), :] = jnp.sum(score, axis=0, keepdims=True)

        return residual, moments, rest

    lane8 = jax.lax.broadcasted_iota(jnp.int32, (8, LANES), 1)
    low8 = lane8 < half
    causal = jax.lax.broadcasted_iota(jnp.int32, (8, LANES), 0) >= lane8 % 8

    def project(lhs, which, p, t, dsts):
        if t < n_main:
            w = jnp.concatenate([_load16(w_v.at[which, p, 2 * t]), _load16(w_v.at[which, p, 2 * t + 1])], axis=1)
        else:
            w = _load16(w_v.at[which, p, 2 * n_main])
        y = jnp.dot(lhs[:, :d_model], w, preferred_element_type=F32)
        for i, (dst, g) in enumerate(dsts):
            yg = y[8 * i:8 * i + 8]
            if t < n_main:
                pair = [yg[:, :LANES], yg[:, LANES:]]
            else:
                pair = [jnp.where(low8, yg, 0.0), jnp.where(low8, 0.0, yg)]
            r0 = g * LANES + 16 * p
            dst[t, r0:r0 + 16, :] = jnp.concatenate(pair, axis=0).astype(BF16)

    def tokens(start, count):
        dsts = [(key_v[(r // seg) % 2], 1 + (r % seg) // 8) for r in range(start, start + count, 8)]
        return h_v[start:start + count, :], dsts

    key_tiles = [(p, t) for t in range(n_tile) for p in range(n_pair)]
    val_tiles = [(p, t) for t in (n_main, *range(n_main)) for p in range(n_pair)]
    ahead = {tile: i % per_blk for i, tile in enumerate(key_tiles[AHEAD_FIRST:AHEAD_FIRST + AHEAD * per_blk])}
    readers = [[rg for rg in range(n_grp) if rg == 0 or rg >= g] for g in range(n_grp)]

    def run_ahead(q, group, lo=0, hi=None):
        lhs, dsts = tokens(q * seg, seg)
        for p, t in [tile for tile, k in ahead.items() if k == group][lo:hi]:
            project(lhs, 0, p, t, dsts)

    def step(q, mem, side):
        keys = key_v[q % 2]
        tok, dsts = tokens(q * seg, seg)
        rows = jnp.concatenate([mem, tok], axis=0)
        side = list(side)
        for i, (p, t) in enumerate(key_tiles):
            if (p, t) in ahead:
                phase = (q - ahead[p, t]) % per_blk
                part, part_dsts = tokens((q + 1) * seg - 8 * phase, seg - 8)
                project(jnp.concatenate([mem, part], axis=0), 0, p, t, [(keys, 0)] + part_dsts)
            else:
                lhs = _after(rows, side.pop(0)()) if side and i >= AHEAD_FIRST else rows
                project(lhs, 0, p, t, [(keys, 0)] + dsts)
        assert not side
        val_dsts = [(val_v, g) for g in range(n_grp)]
        for p, t in val_tiles[:VALUES_EARLY]:
            project(rows, 1, p, t, val_dsts)

        scores = [[jnp.full((8, LANES), -1e9, F32)] * n_grp for _ in range(n_grp)]
        for g in range(n_grp):
            keys_t = jnp.concatenate([_load16(keys.at[t], g * LANES, (g + 1) * LANES).T for t in range(n_tile)],
                                     axis=0)
            sco = jnp.dot(jnp.concatenate([rows[8 * rg:8 * rg + 8] for rg in readers[g]], axis=0), keys_t,
                          preferred_element_type=F32)
            for i, rg in enumerate(readers[g]):
                part = sco[8 * i:8 * i + 8]
                scores[rg][g] = jnp.where(causal, part, -1e9) if 0 < rg == g else part
        probs = []
        for parts in scores:
            top = _group8_allreduce(functools.reduce(jnp.maximum, parts), jnp.maximum, lane8)
            ex = [jnp.exp(part - top) for part in parts]
            inv = 1.0 / _group8_allreduce(functools.reduce(jnp.add, ex), jnp.add, lane8)
            probs.append([e * inv for e in ex])

        for p, t in val_tiles[VALUES_EARLY:]:
            project(rows, 1, p, t, val_dsts)
        acc = [[None] * n_tile for _ in range(n_grp)]
        for t in (n_main, *range(n_main)):
            if t == 1:
                run_ahead(q + 1, (q + 1) % per_blk, 0, 1)
            for g in range(n_grp):
                y = jnp.dot(jnp.concatenate([probs[rg][g] for rg in readers[g]], axis=0),
                            _load16(val_v.at[t], g * LANES, (g + 1) * LANES), preferred_element_type=F32)
                for i, rg in enumerate(readers[g]):
                    part = y[8 * i:8 * i + 8]
                    acc[rg][t] = part if acc[rg][t] is None else acc[rg][t] + part
        out = jnp.concatenate(
            [jnp.concatenate(row[:n_main] + [row[n_main] + pltpu.roll(row[n_main], half, 1)], axis=1)
             for row in acc], axis=0)
        o_v[q * seg:(q + 1) * seg, :] = out[n_mem:]
        run_ahead(q + 1, (q + 1) % per_blk, 1)
        return out[:n_mem]

    def block(b, mem):
        residual, post_moments, post_rest = post(jnp.maximum(b - 1, 0), b - jnp.minimum(b, 1))
        pre_moments, pre_rest = pre(jnp.minimum(b + 1, n_blk - 1), LANES)
        residual()
        mem = step(0, mem, [pre_moments, post_moments])
        post_rest()
        pre_rest()
        for q in range(1, per_blk):
            mem = step(q, mem, [])
        h_v[:LANES] = h_v[LANES:]

        @pl.when(b == 0)
        def _():
            wait(cp_later)
            modulation(later)

        @pl.when(b > 0)
        def _():
            out_copy(b - 1).start()

        return mem

    for job in pre(0, 0):
        job()
    for group in range(per_blk):
        run_ahead(0, group)
    mem0 = mem0_v[...].astype(F32)
    wait(cp_second)
    jax.lax.fori_loop(0, n_blk, block, jnp.concatenate([mem0, mem0[:, d_main:]], axis=1))

    def top1(lo, hi):
        r = _rb(r_v[lo:hi, :])
        r = jnp.where(r != r, -jnp.inf, r)
        best = jnp.max(r, keepdims=True)
        pos = ((jax.lax.broadcasted_iota(jnp.int32, r.shape, 0) + lo) * LANES
               + jax.lax.broadcasted_iota(jnp.int32, r.shape, 1))
        return best, jnp.min(jnp.where(r == best, pos, seq - 1))

    def one_lane(idx):
        return jax.lax.broadcasted_iota(jnp.int32, (d_model, LANES), 1) == idx % LANES

    def ffn(best, idx):
        chosen = jnp.where(one_lane(idx), h2_v[idx // LANES].astype(F32), 0.0).astype(BF16)
        sel = jax.lax.dot_general(jnp.ones((8, LANES), F32), chosen, NT, preferred_element_type=F32)
        gate = _rb(jnp.dot(sel, wg_v[...], preferred_element_type=F32))
        up = _rb(jnp.dot(sel, wu_v[...], preferred_element_type=F32))
        act = _rb(_rb(gate * _rb(jax.nn.sigmoid(gate))) * up)[0:1]
        y = wdt_v[:, :LANES].astype(F32) * act[:, :LANES]
        for lo in range(LANES, act.shape[1], LANES):
            y = y + wdt_v[:, lo:lo + LANES].astype(F32) * act[:, lo:lo + LANES]
        y = _rb(_rb(jnp.sum(y, axis=1, keepdims=True)) * _rb(jax.nn.sigmoid(best)))
        y_v[...] = jnp.broadcast_to(y, y_v.shape)

    wait(cp_ffn)
    best, idx = top1(0, n_blk - 1)
    ffn(best, idx)
    for job in post(n_blk - 1, n_blk - 1):
        job()
    out_copy(n_blk - 1).start()
    best_last, idx_last = top1(n_blk - 1, n_blk)
    replaced = jnp.max(jnp.where(best_last > best, 1, 0)) > 0
    pl.when(replaced)(lambda: ffn(best_last, idx_last))
    idx = jnp.where(replaced, idx_last, idx)

    blk = idx // LANES
    h2 = h2_v[blk].astype(F32)
    zero = h2 * 0.0
    wait([out_copy(b) for b in range(n_blk)])
    out_v[blk] = emit(x1_v[blk], h2, jnp.where(one_lane(idx), zero + y_v[...], zero))
    out_copy(blk).start()
    out_copy(blk).wait()


@functools.partial(jax.jit, static_argnames=("A_seg_len",))
def pallas_adaLN_cond__memory_aug_recurrent_mem_tr__moe_arch_mod__prompt_kernel(
    A_x: jax.Array,
    A_mem0: jax.Array,
    A_Wq: jax.Array,
    A_Wk: jax.Array,
    A_Wv: jax.Array,
    A_Wo: jax.Array,
    A_seg_len: int,
    B_x: jax.Array,
    B_w_r: jax.Array,
    B_w_gate: jax.Array,
    B_w_up: jax.Array,
    B_w_down: jax.Array,
    c: jax.Array,
    w_mod: jax.Array,
):
    del B_x
    _, seq, d_model = A_x.shape
    n_mem = A_mem0.shape[1]
    n_heads, d_head = A_Wq.shape[1:]
    d_ff = B_w_gate.shape[1]
    seg = int(A_seg_len)
    n_blk = seq // LANES
    d_ext = d_model + LANES // 2
    assert A_x.shape[0] == 1 and d_model % LANES == LANES // 2 and d_head % LANES == 0 and d_ff % LANES == 0
    assert n_mem == 8 and n_heads * 8 == LANES and seg == 32 and seq % LANES == 0 and n_blk > 2
    folded = pltpu.VMEM((d_ext // LANES, (n_mem + seg) * n_heads, LANES), BF16)

    hbm = pl.BlockSpec(memory_space=pltpu.HBM)
    out_t = pl.pallas_call(
        functools.partial(_kernel, seg=seg, scale=d_head ** -0.5),
        out_shape=jax.ShapeDtypeStruct((d_model, seq), A_x.dtype),
        in_specs=[hbm] * 12,
        out_specs=hbm,
        scratch_shapes=[
            pltpu.VMEM(c.shape, BF16),
            pltpu.VMEM((n_mem, d_model), BF16),
            pltpu.VMEM(B_w_r.shape, BF16),
            pltpu.VMEM((d_model, seq), BF16),
            pltpu.VMEM((3, n_heads // 2, d_model, d_head), jnp.uint32),
            pltpu.VMEM((n_heads, d_head // LANES, d_model, LANES), BF16),
            pltpu.VMEM((2, n_heads // 2, 2 * d_model // LANES, d_model, LANES), BF16),
            pltpu.VMEM((d_model, d_ff), BF16),
            pltpu.VMEM((d_model, d_ff), BF16),
            pltpu.VMEM((d_model, d_ff), BF16),
            pltpu.VMEM(w_mod.shape, BF16),
            pltpu.VMEM((7, d_model + MOD_PAD, LANES), F32),
            pltpu.VMEM((2 * LANES, d_ext), F32),
            pltpu.VMEM((LANES, d_ext), F32),
            pltpu.VMEM((n_blk, d_model, LANES), F32),
            folded, folded,
            folded,
            pltpu.VMEM((n_blk, LANES), F32),
            pltpu.VMEM((d_model, LANES), F32),
            pltpu.VMEM((n_blk, d_model, LANES), BF16),
            pltpu.VMEM((n_blk, d_model, LANES), BF16),
            pltpu.SemaphoreType.DMA((n_heads + 5,)),
        ],
        compiler_params=pltpu.CompilerParams(vmem_limit_bytes=100 * 1024 * 1024),
    )(c, A_mem0[0], B_w_r, A_x[0].T, A_Wq, A_Wk, A_Wv, jnp.swapaxes(A_Wo, 1, 2),
      B_w_gate, B_w_up, B_w_down.T, w_mod)
    return out_t.T[None]
```
